```python
import jax
import jax.numpy as jnp

def _softmax(x, axis=-1):
    return jax.nn.softmax(x, axis=axis)
def _gelu(x):
    return jax.nn.gelu(x, approximate=True)
def _silu(x):
    return jax.nn.silu(x)
def _sigmoid(x):
    return jax.nn.sigmoid(x)
def _layernorm(x, axis=-1, eps=1e-5):
    m = jnp.mean(x, axis=axis, keepdims=True)
    v = jnp.var(x, axis=axis, keepdims=True)
    return (x - m) / jnp.sqrt(v + eps)
def _scatter_add(tgt, idx, src, axis=0):
    return tgt.at[idx].add(src)
def _segment_sum(src, seg, n):
    return jax.ops.segment_sum(src, seg, n)
class _Rng:
    def __init__(self, key):
        self._k = key
    def _next(self):
        self._k, sub = jax.random.split(self._k)
        return sub
    def normal(self, shape):
        return jax.random.normal(self._next(), shape, dtype=jnp.bfloat16)
    def randint(self, lo, hi, shape):
        return jax.random.randint(self._next(), shape, lo, hi, dtype=jnp.int32)
    def uniform(self, shape, lo=0.0, hi=1.0):
        return jax.random.uniform(self._next(), shape, jnp.bfloat16, lo, hi)
    def permutation(self, n):
        return jax.random.permutation(self._next(), n)


kernel_name = 'recurrent_scan__compressed_kv_cla__moe_arch_mod__decode'

def setup_inputs():
    _rng = _Rng(jax.random.key(int.from_bytes(__import__("os").urandom(4), "little")))
    _w = (lambda a: (lambda t: t.astype(jnp.bfloat16) if jnp.issubdtype(t.dtype, jnp.floating) else t)(jnp.asarray(a)))
    def _A_setup():
        B, H, Sq, Sk, D, M = 4, 32, 1, 4096, 128, 576
        Dc = 4 * D
        return {
            "x": _w((lambda *s: _rng.normal(s) * 0.05)(B, Sq, M)),
            "c_kv": _w((lambda *s: _rng.normal(s) * 0.05)(B, Sk, Dc)),
            "w_q": _w((lambda *s: _rng.normal(s) * 0.05)(M, H, D) * (M ** -0.5)),
            "w_uk": _w((lambda *s: _rng.normal(s) * 0.05)(Dc, H, D) * (Dc ** -0.5)),
            "w_uv": _w((lambda *s: _rng.normal(s) * 0.05)(Dc, H, D) * (Dc ** -0.5)),
            "w_o": _w((lambda *s: _rng.normal(s) * 0.05)(H, D, M) * ((H * D) ** -0.5)),
        }
    _A_in = _A_setup()

    def _B_setup():
        B, S, D, F, C = 4, 1, 576, 4608, 1
        return {
            "x": _w((lambda *s: _rng.normal(s) * 0.05)(B, S, D)),
            "w_r": _w((lambda *s: _rng.normal(s) * 0.05)(D)),
            "w_gate": _w((lambda *s: _rng.normal(s) * 0.05)(D, F)),
            "w_up": _w((lambda *s: _rng.normal(s) * 0.05)(D, F)),
            "w_down": _w((lambda *s: _rng.normal(s) * 0.05)(F, D)),
        }
    _B_in = _B_setup()

    return {
        "A_x": _A_in["x"],
        "A_c_kv": _A_in["c_kv"],
        "A_w_q": _A_in["w_q"],
        "A_w_uk": _A_in["w_uk"],
        "A_w_uv": _A_in["w_uv"],
        "A_w_o": _A_in["w_o"],
        "B_x": _B_in["x"],
        "B_w_r": _B_in["w_r"],
        "B_w_gate": _B_in["w_gate"],
        "B_w_up": _B_in["w_up"],
        "B_w_down": _B_in["w_down"],
    }

def reference(A_x, A_c_kv, A_w_q, A_w_uk, A_w_uv, A_w_o, B_x, B_w_r, B_w_gate, B_w_up, B_w_down):
    def _A_ref(x, c_kv, w_q, w_uk, w_uv, w_o):
        B, Sq, M = x.shape[0], x.shape[1], x.shape[2]
        Sk = c_kv.shape[1]
        H, D = w_q.shape[1], w_q.shape[2]
        q = jnp.einsum("bqm,mhd->bhqd", x, w_q)
        k = jnp.einsum("bkc,chd->bhkd", c_kv, w_uk)
        v = jnp.einsum("bkc,chd->bhkd", c_kv, w_uv)
        scores = jnp.einsum("bhqd,bhkd->bhqk", q, k) * (D ** -0.5)
        off = Sk - Sq
        qi = jnp.arange(Sq)[:, None]
        kj = jnp.arange(Sk)[None, :]
        cmask = kj <= (qi + off)
        scores = jnp.where(cmask[None, None], scores, -1e9)
        p = _softmax(scores, axis=-1)
        ctx = jnp.einsum("bhqk,bhkd->bhqd", p, v)
        return jnp.einsum("bhqd,hdm->bqm", ctx, w_o)

    def _B_ref(x, w_r, w_gate, w_up, w_down):
        B, S, D = x.shape
        C = 1
        r = x @ w_r
        idx = jnp.argsort(-r, axis=-1)[:, :C]
        idx_e = jnp.repeat(idx.reshape(B, C, 1), D, axis=2)
        x_sel = jnp.take_along_axis(x, idx_e, axis=1)
        g = _silu(x_sel @ w_gate)
        u = x_sel @ w_up
        y = (g * u) @ w_down
        r_sel = _sigmoid(jnp.take_along_axis(r, idx, axis=1))
        y = y * r_sel.reshape(B, C, 1)
        b_off = (jnp.arange(B) * S).reshape(B, 1)
        flat_idx = (idx + b_off).reshape(B * C)
        zero = (x * 0.0).reshape(B * S, D)
        upd = _scatter_add(zero, flat_idx, y.reshape(B * C, D), axis=0)
        return x + upd.reshape(B, S, D)

    x = A_x
    xn = _layernorm(x, axis=-1)
    s = _A_ref(xn, A_c_kv, A_w_q, A_w_uk, A_w_uv, A_w_o)
    g = _silu(_B_ref(xn, B_w_r, B_w_gate, B_w_up, B_w_down))
    return x + s * g
```

```python
import functools

import jax
import jax.numpy as jnp
from jax import lax
from jax.experimental import pallas as pl
from jax.experimental.pallas import tpu as pltpu

F32 = jnp.float32
BF16 = jnp.bfloat16
_NT = (((1,), (1,)), ((), ()))


def _dot(a, b):
    return jnp.dot(a, b, preferred_element_type=F32)


def _dot_nt(a, b):
    return lax.dot_general(a, b, _NT, preferred_element_type=F32)


def _sigmoid(z):
    return 1.0 / (1.0 + jnp.exp(-z))


class _NoScope:
    def __enter__(self):
        return self

    def __exit__(self, *a):
        return False


def _kernel(
    x_hbm, ckv_hbm, wq_hbm, wuk_hbm, wuv_hbm, wo_hbm, wr_hbm, wg_hbm, wu_hbm, wd_hbm,
    o_ref,
    x_v, ckv_v, wq_v, wuk_v, wuv_v, wo_v, wr_v, wg_v, wu_v, wd_v,
    e_v, et_v, lq_v, q_v, ql_v, s_v, cl_v, ctx_v, h_v, sems,
    *, wo_chunks, kc, fc, scopes,
):
    B, M = x_v.shape
    _, SK, DC = ckv_v.shape
    _, G, HG, D = wq_v.shape
    H = G * HG
    FF = wg_v.shape[1]
    R = B * HG
    scope = jax.named_scope if scopes else (lambda _: _NoScope())

    cp_x = pltpu.make_async_copy(x_hbm, x_v, sems.at[0])
    cp_wr = pltpu.make_async_copy(wr_hbm, wr_v, sems.at[1])
    cp_wq = pltpu.make_async_copy(wq_hbm, wq_v, sems.at[2])
    cp_wuk = pltpu.make_async_copy(wuk_hbm, wuk_v, sems.at[3])
    cp_ckv = pltpu.make_async_copy(ckv_hbm, ckv_v, sems.at[4])
    cp_wuv = pltpu.make_async_copy(wuv_hbm, wuv_v, sems.at[5])
    cp_wg = pltpu.make_async_copy(wg_hbm, wg_v, sems.at[6])
    cp_wu = pltpu.make_async_copy(wu_hbm, wu_v, sems.at[7])
    cp_wd = pltpu.make_async_copy(wd_hbm, wd_v, sems.at[8])
    cp_wo = []
    h0 = 0
    for i, n in enumerate(wo_chunks):
        cp_wo.append(pltpu.make_async_copy(
            wo_hbm.at[pl.ds(h0, n)], wo_v.at[pl.ds(h0, n)], sems.at[9 + i]))
        h0 += n
    for cp in (cp_x, cp_wr, cp_wq, cp_wuk, cp_ckv, cp_wuv, cp_wg, cp_wu, cp_wd, *cp_wo):
        cp.start()

    with scope("consts"):
        CB = 128
        e_v[...] = (
            lax.broadcasted_iota(jnp.int32, (CB, CB * HG), 1) // HG
            == lax.broadcasted_iota(jnp.int32, (CB, CB * HG), 0)
        ).astype(F32).astype(BF16)
        et_v[...] = (
            lax.broadcasted_iota(jnp.int32, (CB * HG, CB), 0) // HG
            == lax.broadcasted_iota(jnp.int32, (CB * HG, CB), 1)
        ).astype(F32).astype(BF16)

    def same_head(n):
        return (lax.broadcasted_iota(jnp.int32, (R, n), 0) % HG
                == lax.broadcasted_iota(jnp.int32, (R, n), 1) % HG)

    with scope("ln"):
        cp_x.wait()
        x = x_v[...].astype(F32)
        xc = x - jnp.mean(x, axis=1, keepdims=True)
        var = jnp.mean(xc * xc, axis=1, keepdims=True)
        xn = xc / jnp.sqrt(var + 1e-5)
        xn16 = xn.astype(BF16)
        cp_wr.wait()
        wr = wr_v[...].astype(F32).reshape(1, M)
        r_sel = _sigmoid(jnp.sum(xn16.astype(F32) * wr, axis=1, keepdims=True))

        xrep = jnp.concatenate(
            [jnp.broadcast_to(xn[b:b + 1], (HG, M)) for b in range(B)], axis=0
        ).astype(BF16)
        for m0 in range(0, M, CB):
            n = min(CB, M - m0)
            wide = _dot(xrep[:, m0:m0 + n], e_v[0:n, 0:n * HG])
            lq_v[:, m0 * HG:(m0 + n) * HG] = jnp.where(
                same_head(n * HG), wide, 0.0).astype(BF16)

    with scope("wait_wq"):
        cp_wq.wait()
    with scope("q"):
        def q_body(g, _):
            w = wq_v[:, g].reshape(M * HG, D)
            q_v[g] = _dot(lq_v[...], w).astype(BF16)
        lax.fori_loop(0, G, q_body, None)

    with scope("wait_wuk"):
        cp_wuk.wait()
    with scope("qlat"):
        def ql_body(i, _):
            g = i // (DC // CB)
            c0 = pl.multiple_of((i % (DC // CB)) * CB, CB)
            w = wuk_v[pl.ds(c0, CB), g].reshape(CB * HG, D)
            wide = _dot_nt(q_v[g], w)
            wide = jnp.where(same_head(CB * HG), wide, 0.0).astype(BF16)
            ql = _dot(wide, et_v[...])
            for b in range(B):
                ql_v[b, g, :, pl.ds(c0, CB)] = ql[b * HG:(b + 1) * HG]
        lax.fori_loop(0, G * (DC // CB), ql_body, None)

    with scope("wait_ckv"):
        cp_ckv.wait()
    with scope("attn"):
        scale = D ** -0.5

        def attn_body(b, _):
            ql = ql_v[b].reshape(H, DC).astype(BF16)

            def s_body(j, m):
                k0 = pl.multiple_of(j * kc, kc)
                s = _dot_nt(ql, ckv_v[b, pl.ds(k0, kc), :]) * scale
                s_v[:, pl.ds(k0, kc)] = s
                for t in range(kc // 128):
                    m = jnp.maximum(m, s[:, t * 128:(t + 1) * 128])
                return m
            m = lax.fori_loop(0, SK // kc, s_body, jnp.full((H, 128), -jnp.inf, F32))
            m = jnp.max(m, axis=1, keepdims=True)

            def pv_body(j, carry):
                l, acc = carry
                k0 = pl.multiple_of(j * kc, kc)
                p = jnp.exp(s_v[:, pl.ds(k0, kc)] - m)
                for t in range(kc // 128):
                    l = l + p[:, t * 128:(t + 1) * 128]
                acc = acc + _dot(p.astype(BF16), ckv_v[b, pl.ds(k0, kc), :])
                return l, acc
            l, acc = lax.fori_loop(
                0, SK // kc, pv_body,
                (jnp.zeros((H, 128), F32), jnp.zeros((H, DC), F32)))
            cl = acc / jnp.sum(l, axis=1, keepdims=True)
            for g in range(G):
                cl_v[g, b] = cl[g * HG:(g + 1) * HG]
        lax.fori_loop(0, B, attn_body, None)

    with scope("wait_wuv"):
        cp_wuv.wait()
    with scope("ctx"):
        pr = lax.broadcasted_iota(jnp.int32, (HG * 8, R), 0)
        pc = lax.broadcasted_iota(jnp.int32, (HG * 8, R), 1)
        perm = jnp.logical_and(pr // 8 == pc % HG, pr % 8 == pc // HG).astype(F32).astype(BF16)

        def ctx_body(g, _):
            def blk(j, acc):
                c0 = pl.multiple_of(j * CB, CB)
                cl = cl_v[g, :, :, pl.ds(c0, CB)].reshape(R, CB).astype(BF16)
                wide = _dot(cl, e_v[...])
                wide = jnp.where(same_head(CB * HG), wide, 0.0).astype(BF16)
                w = wuv_v[pl.ds(c0, CB), g].reshape(CB * HG, D)
                return acc + _dot(wide, w)
            ctx = lax.fori_loop(0, DC // CB, blk, jnp.zeros((R, D), F32))
            ctx_v[g] = _dot(perm, ctx.astype(BF16)).reshape(HG, 8, D)
        lax.fori_loop(0, G, ctx_body, None)

    with scope("wait_wgu"):
        cp_wg.wait()
        cp_wu.wait()
    with scope("gateup"):
        def up_body(j, _):
            f0 = pl.multiple_of(j * fc, fc)
            gt = _dot(xn16, wg_v[:, pl.ds(f0, fc)])
            up = _dot(xn16, wu_v[:, pl.ds(f0, fc)])
            h_v[:, pl.ds(f0, fc)] = gt * _sigmoid(gt) * up
        lax.fori_loop(0, FF // fc, up_body, None)

    with scope("wait_wd"):
        cp_wd.wait()
    with scope("down"):
        def down_body(j, y):
            f0 = pl.multiple_of(j * fc, fc)
            return y + _dot_nt(h_v[:, pl.ds(f0, fc)].astype(BF16), wd_v[:, pl.ds(f0, fc)])
        y = lax.fori_loop(0, FF // fc, down_body, jnp.zeros((B, M), F32))
        z = xn + (xn * 0.0 + y * r_sel)
        gate = z * _sigmoid(z)

    def o_body(h, s):
        ctx = ctx_v[h // HG, h % HG].astype(BF16)
        return s + _dot_nt(ctx, wo_v[h])

    s = jnp.zeros((8, M), F32)
    h0 = 0
    for i, (cp, n) in enumerate(zip(cp_wo, wo_chunks)):
        with scope(f"wait_wo{i}"):
            cp.wait()
        with scope(f"wo{i}"):
            if n == 1:
                s = o_body(h0, s)
            else:
                s = lax.fori_loop(h0, h0 + n, o_body, s)
        h0 += n
    o_ref[...] = (x + s[0:B] * gate).astype(o_ref.dtype)


def make(wo_chunks=(20, 8, 3, 1), kc=512, fc=512, scopes=False, interpret=False):
    def f(A_x, A_c_kv, A_w_q, A_w_uk, A_w_uv, A_w_o, B_x, B_w_r, B_w_gate, B_w_up, B_w_down):
        del B_x
        B, _, M = A_x.shape
        _, SK, DC = A_c_kv.shape
        _, H, D = A_w_q.shape
        FF = B_w_gate.shape[1]
        HG = 8
        G = H // HG
        args = (
            A_x.reshape(B, M),
            A_c_kv,
            A_w_q.reshape(M, G, HG, D),
            A_w_uk.reshape(DC, G, HG, D),
            A_w_uv.reshape(DC, G, HG, D),
            jnp.transpose(A_w_o, (0, 2, 1)),
            B_w_r,
            B_w_gate,
            B_w_up,
            B_w_down.T,
        )
        R = B * HG
        out = pl.pallas_call(
            functools.partial(_kernel, wo_chunks=wo_chunks, kc=kc, fc=fc, scopes=scopes),
            in_specs=[pl.BlockSpec(memory_space=pltpu.HBM)] * len(args),
            out_specs=pl.BlockSpec(memory_space=pltpu.VMEM),
            out_shape=jax.ShapeDtypeStruct((B, M), A_x.dtype),
            scratch_shapes=[pltpu.VMEM(a.shape, a.dtype) for a in args] + [
                pltpu.VMEM((128, 128 * HG), BF16),
                pltpu.VMEM((128 * HG, 128), BF16),
                pltpu.VMEM((R, M * HG), BF16),
                pltpu.VMEM((G, R, D), BF16),
                pltpu.VMEM((B, G, HG, DC), F32),
                pltpu.VMEM((H, SK), F32),
                pltpu.VMEM((G, B, HG, DC), F32),
                pltpu.VMEM((G, HG, 8, D), F32),
                pltpu.VMEM((B, FF), F32),
                pltpu.SemaphoreType.DMA((9 + len(wo_chunks),)),
            ],
            compiler_params=pltpu.CompilerParams(vmem_limit_bytes=100 * 2**20),
            interpret=interpret,
        )(*args)
        return out.reshape(A_x.shape)
    return f


_impl = make()


@jax.jit
def pallas_recurrent_scan__compressed_kv_cla__moe_arch_mod__decode_kernel(
    A_x: jax.Array,
    A_c_kv: jax.Array,
    A_w_q: jax.Array,
    A_w_uk: jax.Array,
    A_w_uv: jax.Array,
    A_w_o: jax.Array,
    B_x: jax.Array,
    B_w_r: jax.Array,
    B_w_gate: jax.Array,
    B_w_up: jax.Array,
    B_w_down: jax.Array,
):
    return _impl(A_x, A_c_kv, A_w_q, A_w_uk, A_w_uv, A_w_o, B_x, B_w_r, B_w_gate, B_w_up, B_w_down)
```

```python
import functools

import jax
import jax.numpy as jnp
from jax import lax
from jax.experimental import pallas as pl
from jax.experimental.pallas import tpu as pltpu

F32 = jnp.float32
BF16 = jnp.bfloat16
LANES = 128
HG = 8
KEYS = 512
COLS = 512


def _dot(a, b):
    return jnp.dot(a, b, preferred_element_type=F32)


def _dot_t(a, b):
    return lax.dot_general(a, b, (((1,), (1,)), ((), ())), preferred_element_type=F32)


def _iota(shape, axis):
    return lax.broadcasted_iota(jnp.int32, shape, axis)


def _indicator(cond):
    return cond.astype(F32).astype(BF16)


def _kernel(
    x_hbm, ckv_hbm, wq_hbm, wuk_hbm, wuv_hbm, wo_hbm, wr_hbm, wg_hbm, wu_hbm, wd_hbm,
    out_hbm,
    x_v, ckv_v, wq_v, wuk_v, wuv_v, wo_v, wr_v, wg_v, wu_v, wd_v,
    spread_v, gather_v, xq_v, q_v, ql_v, score_v, cl_v, ctx_v, hid_v, out_v,
    *, wo_pieces, manual_out,
):
    B, M = x_v.shape
    _, SK, DC = ckv_v.shape
    _, G, _, D = wq_v.shape
    FF = wg_v.shape[1]
    H = G * HG
    R = B * HG
    NT = pl.cdiv(M, LANES)

    def own_head(v):
        return jnp.where(
            _iota(v.shape, 0) % HG == _iota(v.shape, 1) % HG, v, 0.0
        ).astype(BF16)

    def layernorm_and_router(cp_x, cp_wr):
        cp_x.wait()
        x = x_v[...].astype(F32)
        xc = x - jnp.mean(x, axis=1, keepdims=True)
        var = jnp.mean(xc * xc, axis=1, keepdims=True)
        xn = xc / jnp.sqrt(var + 1e-5)
        cp_wr.wait()
        wr = wr_v[...].astype(F32).reshape(1, M)
        route = jax.nn.sigmoid(jnp.sum(xn * wr, axis=1, keepdims=True))
        return x, xn, route

    def queries(xn, cp_wq):
        xr = jnp.concatenate(
            [jnp.broadcast_to(xn[b:b + 1], (HG, M)) for b in range(B)], axis=0
        ).astype(BF16)
        for m0 in range(0, M, LANES):
            n = min(LANES, M - m0)
            xq_v[:, m0 * HG:(m0 + n) * HG] = own_head(
                _dot(xr[:, m0:m0 + n], spread_v[0:n, 0:n * HG]))
        cp_wq.wait()

        @pl.loop(0, G)
        def _(g):
            q_v[g] = _dot(xq_v[...], wq_v[:, g].reshape(M * HG, D)).astype(BF16)

    def latent_queries():
        @pl.loop(0, G * (DC // LANES))
        def _(i):
            g = i // (DC // LANES)
            c = pl.ds(pl.multiple_of(i % (DC // LANES) * LANES, LANES), LANES)
            wide = own_head(_dot_t(q_v[g], wuk_v[c, g].reshape(LANES * HG, D)))
            ql = _dot(wide, gather_v[...])
            for b in range(B):
                ql_v[b, g, :, c] = ql[b * HG:(b + 1) * HG]

    def attention():
        @pl.loop(0, B)
        def _(b):
            ql = ql_v[b].reshape(H, DC).astype(BF16)

            def scores(j, top):
                k = pl.ds(pl.multiple_of(j * KEYS, KEYS), KEYS)
                s = _dot_t(ql, ckv_v[b, k, :]) * D ** -0.5
                score_v[:, k] = s
                for t in range(0, KEYS, LANES):
                    top = jnp.maximum(top, s[:, t:t + LANES])
                return top

            top = lax.fori_loop(0, SK // KEYS, scores, jnp.full((H, LANES), -jnp.inf, F32))
            top = jnp.max(top, axis=1, keepdims=True)

            def values(j, carry):
                total, acc = carry
                k = pl.ds(pl.multiple_of(j * KEYS, KEYS), KEYS)
                p = jnp.exp(score_v[:, k] - top)
                for t in range(0, KEYS, LANES):
                    total = total + p[:, t:t + LANES]
                return total, acc + _dot(p.astype(BF16), ckv_v[b, k, :])

            total, acc = lax.fori_loop(
                0, SK // KEYS, values,
                (jnp.zeros((H, LANES), F32), jnp.zeros((H, DC), F32)))
            cl = acc / jnp.sum(total, axis=1, keepdims=True)
            for g in range(G):
                cl_v[g, b] = cl[g * HG:(g + 1) * HG]

    def contexts():
        row, col = _iota((HG * 8, R), 0), _iota((HG * 8, R), 1)
        by_head = _indicator(jnp.logical_and(row // 8 == col % HG, row % 8 == col // HG))

        @pl.loop(0, G)
        def _(g):
            def block(j, acc):
                c = pl.ds(pl.multiple_of(j * LANES, LANES), LANES)
                cl = cl_v[g, :, :, c].reshape(R, LANES).astype(BF16)
                wide = own_head(_dot(cl, spread_v[...]))
                return acc + _dot(wide, wuv_v[c, g].reshape(LANES * HG, D))

            ctx = lax.fori_loop(0, DC // LANES, block, jnp.zeros((R, D), F32))
            ctx_v[pl.ds(g * HG, HG)] = _dot(by_head, ctx.astype(BF16)).reshape(HG, 8, D)

    def hidden(xn):
        xn = xn.astype(BF16)

        @pl.loop(0, FF // COLS)
        def _(j):
            f = pl.ds(pl.multiple_of(j * COLS, COLS), COLS)
            hid_v[:, f] = jax.nn.silu(_dot(xn, wg_v[:, f])) * _dot(xn, wu_v[:, f])

    def gate(xn, route):
        def block(j, y):
            f = pl.ds(pl.multiple_of(j * COLS, COLS), COLS)
            return y + _dot_t(hid_v[:, f].astype(BF16), wd_v[:, f])

        y = lax.fori_loop(0, FF // COLS, block, jnp.zeros((B, M), F32))
        return jax.nn.silu(xn + (xn * 0.0 + y * route))

    def project(h, t0, t1, s):
        m0, m1 = t0 * LANES, min(t1 * LANES, M)
        row = h * M + m0
        if not isinstance(row, int):
            row = pl.multiple_of(row, 64)
        part = _dot_t(ctx_v[h].astype(BF16), wo_v[pl.ds(row, m1 - m0), :])
        return tuple(
            s[t] + part[:, t * LANES - m0:min((t + 1) * LANES, M) - m0]
            if t0 <= t < t1 else s[t]
            for t in range(NT))

    def project_piece(u0, u1, s):
        def heads(h, n, s):
            for i in range(n):
                s = project(h + i, 0, NT, s)
            return s

        h = pl.cdiv(u0, NT)
        if u0 % NT:
            s = project(h - 1, u0 % NT, min(NT, u1 - (h - 1) * NT), s)
        n = max(u1 // NT - h, 0)
        if n >= 8:
            s = lax.fori_loop(0, n // 4, lambda j, s, h=h: heads(h + 4 * j, 4, s), s)
            h, n = h + n // 4 * 4, n % 4
        s = heads(h, n, s)
        if (h + n) * NT < u1:
            s = project(h + n, 0, u1 - (h + n) * NT, s)
        return s

    def run(sems):
        whole = [
            (wq_hbm, wq_v), (x_hbm, x_v), (wr_hbm, wr_v), (wuk_hbm, wuk_v), (ckv_hbm, ckv_v),
            (wuv_hbm, wuv_v), (wg_hbm, wg_v), (wu_hbm, wu_v), (wd_hbm, wd_v)]
        for u0, u1 in wo_pieces:
            r0, r1 = (u // NT * M + u % NT * LANES for u in (u0, u1))
            whole.append((wo_hbm.at[pl.ds(r0, r1 - r0)], wo_v.at[pl.ds(r0, r1 - r0)]))
        copies = [
            pltpu.make_async_copy(src, dst, sems.at[i]) for i, (src, dst) in enumerate(whole)]
        for cp in copies:
            cp.start()
        cp_wq, cp_x, cp_wr, cp_wuk, cp_ckv, cp_wuv, cp_wg, cp_wu, cp_wd, *cp_wo = copies

        spread_v[...] = _indicator(_iota(spread_v.shape, 1) // HG == _iota(spread_v.shape, 0))
        gather_v[...] = _indicator(_iota(gather_v.shape, 0) // HG == _iota(gather_v.shape, 1))

        x, xn, route = layernorm_and_router(cp_x, cp_wr)
        queries(xn, cp_wq)
        cp_wuk.wait()
        latent_queries()
        cp_ckv.wait()
        attention()
        cp_wuv.wait()
        contexts()
        cp_wg.wait()
        cp_wu.wait()
        hidden(xn)
        cp_wd.wait()
        g = gate(xn, route)

        zero = tuple(jnp.zeros((8, min(LANES, M - t * LANES)), F32) for t in range(NT))
        s = zero
        for cp, piece in zip(cp_wo[:-1], wo_pieces[:-1]):
            cp.wait()
            s = project_piece(*piece, s)
        x, g = (jnp.concatenate([v] * (8 // B), axis=0) for v in (x, g))
        out = x + jnp.concatenate(s, axis=1) * g
        cp_wo[-1].wait()
        s = project_piece(*wo_pieces[-1], zero)
        out = out + jnp.concatenate(s, axis=1) * g
        if manual_out:
            out_v[...] = out.astype(out_v.dtype)[0:B]
            cp = pltpu.make_async_copy(out_v, out_hbm, sems.at[len(copies)])
            cp.start()
            cp.wait()
        else:
            out_hbm[...] = out.astype(out_v.dtype)[0:B]

    pl.run_scoped(run, pltpu.SemaphoreType.DMA((10 + len(wo_pieces),)))


def make(tail=(20, 10, 5, 5), wrap=4, manual_out=True):
    def f(A_x, A_c_kv, A_w_q, A_w_uk, A_w_uv, A_w_o, B_x, B_w_r, B_w_gate, B_w_up, B_w_down):
        del B_x
        B, _, M = A_x.shape
        _, SK, DC = A_c_kv.shape
        _, H, D = A_w_q.shape
        FF = B_w_gate.shape[1]
        G, R = H // HG, B * HG
        ends = [H * pl.cdiv(M, LANES)]
        for n in reversed(tail):
            ends.insert(0, ends[0] - n)
        wo_pieces = (*zip([wrap, *ends[:-1]], ends), (0, wrap))
        args = (
            A_x.reshape(B, M),
            A_c_kv,
            A_w_q.reshape(M, G, HG, D),
            A_w_uk.reshape(DC, G, HG, D),
            A_w_uv.reshape(DC, G, HG, D),
            jnp.transpose(A_w_o, (0, 2, 1)).reshape(H * M, D),
            B_w_r,
            B_w_gate,
            B_w_up,
            B_w_down.T,
        )
        out = pl.pallas_call(
            functools.partial(_kernel, wo_pieces=wo_pieces, manual_out=manual_out),
            in_specs=[pl.BlockSpec(memory_space=pltpu.HBM)] * len(args),
            out_specs=pl.BlockSpec(memory_space=pltpu.HBM if manual_out else pltpu.VMEM),
            out_shape=jax.ShapeDtypeStruct((B, M), A_x.dtype),
            scratch_shapes=[pltpu.VMEM(a.shape, a.dtype) for a in args] + [
                pltpu.VMEM((LANES, LANES * HG), BF16),
                pltpu.VMEM((LANES * HG, LANES), BF16),
                pltpu.VMEM((R, M * HG), BF16),
                pltpu.VMEM((G, R, D), BF16),
                pltpu.VMEM((B, G, HG, DC), F32),
                pltpu.VMEM((H, SK), F32),
                pltpu.VMEM((G, B, HG, DC), F32),
                pltpu.VMEM((H, 8, D), F32),
                pltpu.VMEM((B, FF), F32),
                pltpu.VMEM((B, M), A_x.dtype),
            ],
            compiler_params=pltpu.CompilerParams(vmem_limit_bytes=80 * 2**20),
        )(*args)
        return out.reshape(A_x.shape)
    return f


_impl = make(tail=(40, 20, 10, 5, 5))


@jax.jit
def pallas_recurrent_scan__compressed_kv_cla__moe_arch_mod__decode_kernel(
    A_x: jax.Array,
    A_c_kv: jax.Array,
    A_w_q: jax.Array,
    A_w_uk: jax.Array,
    A_w_uv: jax.Array,
    A_w_o: jax.Array,
    B_x: jax.Array,
    B_w_r: jax.Array,
    B_w_gate: jax.Array,
    B_w_up: jax.Array,
    B_w_down: jax.Array,
):
    return _impl(A_x, A_c_kv, A_w_q, A_w_uk, A_w_uv, A_w_o, B_x, B_w_r, B_w_gate, B_w_up, B_w_down)
```

```python
import functools

import jax
import jax.numpy as jnp
from jax import lax
import jax.experimental.pallas as pl
import jax.experimental.pallas.tpu as pltpu

F32 = jnp.float32
BF16 = jnp.bfloat16
LANES = 128
HG = 8
KEYS = 512
COLS = 512
WO_TAIL = (40, 20, 10, 5, 5)
WO_LAST = 4


def _dot(a, b):
    return jnp.dot(a, b, preferred_element_type=F32)


def _dot_t(a, b):
    return lax.dot_general(a, b, (((1,), (1,)), ((), ())), preferred_element_type=F32)


def _iota(shape, axis):
    return lax.broadcasted_iota(jnp.int32, shape, axis)


def _indicator(cond):
    return cond.astype(F32).astype(BF16)


def _kernel(
    x_hbm, ckv_hbm, wq_hbm, wuk_hbm, wuv_hbm, wo_hbm, wr_hbm, wg_hbm, wu_hbm, wd_hbm,
    out_ref,
    x_v, ckv_v, wq_v, wuk_v, wuv_v, wo_v, wr_v, wg_v, wu_v, wd_v,
    spread_v, gather_v, xq_v, q_v, ql_v, score_v, cl_v, ctx_v, hid_v,
    *, wo_pieces,
):
    B, M = x_v.shape
    _, SK, DC = ckv_v.shape
    _, G, _, D = wq_v.shape
    FF = wg_v.shape[1]
    H = G * HG
    R = B * HG
    NT = pl.cdiv(M, LANES)

    def own_head(v):
        return jnp.where(
            _iota(v.shape, 0) % HG == _iota(v.shape, 1) % HG, v, 0.0
        ).astype(BF16)

    def layernorm_and_router(cp_x, cp_wr):
        cp_x.wait()
        x = x_v[...].astype(F32)
        xc = x - jnp.mean(x, axis=1, keepdims=True)
        var = jnp.mean(xc * xc, axis=1, keepdims=True)
        xn = xc / jnp.sqrt(var + 1e-5)
        cp_wr.wait()
        wr = wr_v[...].astype(F32).reshape(1, M)
        route = jax.nn.sigmoid(jnp.sum(xn * wr, axis=1, keepdims=True))
        return x, xn, route

    def queries(xn, cp_wq):
        xr = jnp.concatenate(
            [jnp.broadcast_to(xn[b:b + 1], (HG, M)) for b in range(B)], axis=0
        ).astype(BF16)
        for m0 in range(0, M, LANES):
            n = min(LANES, M - m0)
            xq_v[:, m0 * HG:(m0 + n) * HG] = own_head(
                _dot(xr[:, m0:m0 + n], spread_v[0:n, 0:n * HG]))
        cp_wq.wait()

        @pl.loop(0, G)
        def _(g):
            q_v[g] = _dot(xq_v[...], wq_v[:, g].reshape(M * HG, D)).astype(BF16)

    def latent_queries():
        @pl.loop(0, G * (DC // LANES))
        def _(i):
            g = i // (DC // LANES)
            c = pl.ds(pl.multiple_of(i % (DC // LANES) * LANES, LANES), LANES)
            wide = own_head(_dot_t(q_v[g], wuk_v[c, g].reshape(LANES * HG, D)))
            ql = _dot(wide, gather_v[...])
            for b in range(B):
                ql_v[b, g, :, c] = ql[b * HG:(b + 1) * HG]

    def attention():
        @pl.loop(0, B)
        def _(b):
            ql = ql_v[b].reshape(H, DC).astype(BF16)

            def scores(j, top):
                k = pl.ds(pl.multiple_of(j * KEYS, KEYS), KEYS)
                s = _dot_t(ql, ckv_v[b, k, :]) * D ** -0.5
                score_v[:, k] = s
                for t in range(0, KEYS, LANES):
                    top = jnp.maximum(top, s[:, t:t + LANES])
                return top

            top = lax.fori_loop(
                0, SK // KEYS, scores, jnp.full((H, LANES), -jnp.inf, F32))
            top = jnp.max(top, axis=1, keepdims=True)

            def values(j, carry):
                total, acc = carry
                k = pl.ds(pl.multiple_of(j * KEYS, KEYS), KEYS)
                p = jnp.exp(score_v[:, k] - top)
                for t in range(0, KEYS, LANES):
                    total = total + p[:, t:t + LANES]
                return total, acc + _dot(p.astype(BF16), ckv_v[b, k, :])

            total, acc = lax.fori_loop(
                0, SK // KEYS, values,
                (jnp.zeros((H, LANES), F32), jnp.zeros((H, DC), F32)))
            cl = acc / jnp.sum(total, axis=1, keepdims=True)
            for g in range(G):
                cl_v[g, b] = cl[g * HG:(g + 1) * HG]

    def contexts():
        row, col = _iota((HG * 8, R), 0), _iota((HG * 8, R), 1)
        by_head = _indicator(
            jnp.logical_and(row // 8 == col % HG, row % 8 == col // HG))

        @pl.loop(0, G)
        def _(g):
            def block(j, acc):
                c = pl.ds(pl.multiple_of(j * LANES, LANES), LANES)
                cl = cl_v[g, :, :, c].reshape(R, LANES).astype(BF16)
                wide = own_head(_dot(cl, spread_v[...]))
                return acc + _dot(wide, wuv_v[c, g].reshape(LANES * HG, D))

            ctx = lax.fori_loop(0, DC // LANES, block, jnp.zeros((R, D), F32))
            ctx_v[pl.ds(g * HG, HG)] = _dot(by_head, ctx.astype(BF16)).reshape(HG, 8, D)

    def hidden(xn):
        xn = xn.astype(BF16)

        @pl.loop(0, FF // COLS)
        def _(j):
            f = pl.ds(pl.multiple_of(j * COLS, COLS), COLS)
            hid_v[:, f] = jax.nn.silu(_dot(xn, wg_v[:, f])) * _dot(xn, wu_v[:, f])

    def gate(xn, route):
        def block(j, y):
            f = pl.ds(pl.multiple_of(j * COLS, COLS), COLS)
            return y + _dot_t(hid_v[:, f].astype(BF16), wd_v[:, f])

        y = lax.fori_loop(0, FF // COLS, block, jnp.zeros((B, M), F32))
        return jax.nn.silu(xn + (xn * 0.0 + y * route))

    def project(h, t0, t1, s):
        m0, m1 = t0 * LANES, min(t1 * LANES, M)
        row = h * M + m0
        if not isinstance(row, int):
            row = pl.multiple_of(row, 64)
        part = _dot_t(ctx_v[h].astype(BF16), wo_v[pl.ds(row, m1 - m0), :])
        return tuple(
            s[t] + part[:, t * LANES - m0:min((t + 1) * LANES, M) - m0]
            if t0 <= t < t1 else s[t]
            for t in range(NT))

    def project_piece(u0, u1, s):
        def heads(h, n, s):
            for i in range(n):
                s = project(h + i, 0, NT, s)
            return s

        h = pl.cdiv(u0, NT)
        if u0 % NT:
            s = project(h - 1, u0 % NT, min(NT, u1 - (h - 1) * NT), s)
        n = max(u1 // NT - h, 0)
        if n >= 8:
            s = lax.fori_loop(0, n // 4, lambda j, s, h=h: heads(h + 4 * j, 4, s), s)
            h, n = h + n // 4 * 4, n % 4
        s = heads(h, n, s)
        if (h + n) * NT < u1:
            s = project(h + n, 0, u1 - (h + n) * NT, s)
        return s

    def run(sems):
        reads = [
            (wq_hbm, wq_v), (x_hbm, x_v), (wr_hbm, wr_v), (wuk_hbm, wuk_v),
            (ckv_hbm, ckv_v), (wuv_hbm, wuv_v), (wg_hbm, wg_v), (wu_hbm, wu_v),
            (wd_hbm, wd_v)]
        for piece in wo_pieces:
            r0, r1 = (u // NT * M + u % NT * LANES for u in piece)
            reads.append((wo_hbm.at[pl.ds(r0, r1 - r0)], wo_v.at[pl.ds(r0, r1 - r0)]))
        copies = [
            pltpu.make_async_copy(src, dst, sems.at[i])
            for i, (src, dst) in enumerate(reads)]
        for cp in copies:
            cp.start()
        cp_wq, cp_x, cp_wr, cp_wuk, cp_ckv, cp_wuv, cp_wg, cp_wu, cp_wd, *cp_wo = copies

        spread_v[...] = _indicator(
            _iota(spread_v.shape, 1) // HG == _iota(spread_v.shape, 0))
        gather_v[...] = _indicator(
            _iota(gather_v.shape, 0) // HG == _iota(gather_v.shape, 1))

        x, xn, route = layernorm_and_router(cp_x, cp_wr)
        queries(xn, cp_wq)
        cp_wuk.wait()
        latent_queries()
        cp_ckv.wait()
        attention()
        cp_wuv.wait()
        contexts()
        cp_wg.wait()
        cp_wu.wait()
        hidden(xn)
        cp_wd.wait()
        g = gate(xn, route)

        zero = tuple(jnp.zeros((8, min(LANES, M - t * LANES)), F32) for t in range(NT))
        s = zero
        for cp, piece in zip(cp_wo[:-1], wo_pieces[:-1]):
            cp.wait()
            s = project_piece(*piece, s)
        x, g = (jnp.concatenate([v] * (8 // B), axis=0) for v in (x, g))
        out = x + jnp.concatenate(s, axis=1) * g
        cp_wo[-1].wait()
        s = project_piece(*wo_pieces[-1], zero)
        out = out + jnp.concatenate(s, axis=1) * g
        out_ref[...] = out.astype(out_ref.dtype)[0:B]

    pl.run_scoped(run, pltpu.SemaphoreType.DMA((9 + len(wo_pieces),)))


@jax.jit
def pallas_recurrent_scan__compressed_kv_cla__moe_arch_mod__decode_kernel(
    A_x: jax.Array,
    A_c_kv: jax.Array,
    A_w_q: jax.Array,
    A_w_uk: jax.Array,
    A_w_uv: jax.Array,
    A_w_o: jax.Array,
    B_x: jax.Array,
    B_w_r: jax.Array,
    B_w_gate: jax.Array,
    B_w_up: jax.Array,
    B_w_down: jax.Array,
):
    del B_x
    B, _, M = A_x.shape
    _, SK, DC = A_c_kv.shape
    _, H, D = A_w_q.shape
    FF = B_w_gate.shape[1]
    G, R = H // HG, B * HG
    assert A_x.shape[1] == 1 and 8 % B == 0 and M % 64 == 0

    ends = [H * pl.cdiv(M, LANES)]
    for n in reversed(WO_TAIL):
        ends.insert(0, ends[0] - n)
    wo_pieces = (*zip([WO_LAST, *ends[:-1]], ends), (0, WO_LAST))

    args = (
        A_x.reshape(B, M),
        A_c_kv,
        A_w_q.reshape(M, G, HG, D),
        A_w_uk.reshape(DC, G, HG, D),
        A_w_uv.reshape(DC, G, HG, D),
        jnp.transpose(A_w_o, (0, 2, 1)).reshape(H * M, D),
        B_w_r,
        B_w_gate,
        B_w_up,
        B_w_down.T,
    )
    out = pl.pallas_call(
        functools.partial(_kernel, wo_pieces=wo_pieces),
        in_specs=[pl.BlockSpec(memory_space=pltpu.HBM)] * len(args),
        out_specs=pl.BlockSpec(memory_space=pltpu.VMEM),
        out_shape=jax.ShapeDtypeStruct((B, M), A_x.dtype),
        scratch_shapes=[pltpu.VMEM(a.shape, a.dtype) for a in args] + [
            pltpu.VMEM((LANES, LANES * HG), BF16),
            pltpu.VMEM((LANES * HG, LANES), BF16),
            pltpu.VMEM((R, M * HG), BF16),
            pltpu.VMEM((G, R, D), BF16),
            pltpu.VMEM((B, G, HG, DC), F32),
            pltpu.VMEM((H, SK), F32),
            pltpu.VMEM((G, B, HG, DC), F32),
            pltpu.VMEM((H, 8, D), F32),
            pltpu.VMEM((B, FF), F32),
        ],
        compiler_params=pltpu.CompilerParams(vmem_limit_bytes=80 * 2**20),
    )(*args)
    return out.reshape(A_x.shape)
```
